```python
import os as _os
_os.environ.setdefault("JAX_PLATFORMS", "cpu")
import jax
import jax.numpy as jnp

def _softmax(x, axis=-1):
    return jax.nn.softmax(x, axis=axis)
def _gelu(x):
    return jax.nn.gelu(x, approximate=True)
def _silu(x):
    return jax.nn.silu(x)
def _sigmoid(x):
    return jax.nn.sigmoid(x)
def _layernorm(x, axis=-1, eps=1e-5):
    m = jnp.mean(x, axis=axis, keepdims=True)
    v = jnp.var(x, axis=axis, keepdims=True)
    return (x - m) / jnp.sqrt(v + eps)
def _scatter_add(tgt, idx, src, axis=0):
    return tgt.at[idx].add(src)
def _segment_sum(src, seg, n):
    return jax.ops.segment_sum(src, seg, n)
class _Rng:
    def __init__(self, key):
        self._k = key
    def _next(self):
        self._k, sub = jax.random.split(self._k)
        return sub
    def normal(self, shape):
        return jax.random.normal(self._next(), shape, dtype=jnp.bfloat16)
    def randint(self, lo, hi, shape):
        return jax.random.randint(self._next(), shape, lo, hi, dtype=jnp.int32)
    def uniform(self, shape, lo=0.0, hi=1.0):
        return jax.random.uniform(self._next(), shape, jnp.bfloat16, lo, hi)
    def permutation(self, n):
        return jax.random.permutation(self._next(), n)


kernel_name = 'standalone__mha_softmax__near_ridge'

def setup_inputs():
    _rng = _Rng(jax.random.key(int.from_bytes(__import__("os").urandom(4), "little")))
    _w = (lambda a: (lambda t: t.astype(jnp.bfloat16) if jnp.issubdtype(t.dtype, jnp.floating) else t)(jnp.asarray(a)))
    B, H, Sq, Sk, D = 16, 16, 256, 256, 256
    return {
        "q": _w((lambda *s: _rng.normal(s) * 0.4)(B, H, Sq, D)),
        "k": _w((lambda *s: _rng.normal(s) * 0.4)(B, H, Sk, D)),
        "v": _w((lambda *s: _rng.normal(s) * 0.05)(B, H, Sk, D)),
    }

def reference(q, k, v):
    scale = q.shape[-1] ** -0.5
    scores = jnp.einsum("bhqd,bhkd->bhqk", q, k) * scale
    p = _softmax(scores, axis=-1)
    return jnp.einsum("bhqk,bhkd->bhqd", p, v)
```

```python
import functools

import jax
import jax.numpy as jnp
import jax.experimental.pallas as pl
import jax.experimental.pallas.tpu as pltpu


def _mha_kernel(q_ref, k_ref, v_ref, o_ref, *, hb, scale):
    for h in range(hb):
        q = q_ref[h]
        k = k_ref[h]
        v = v_ref[h]
        s = jax.lax.dot_general(
            q, k, (((1,), (1,)), ((), ())), preferred_element_type=jnp.float32
        ) * scale
        m = jnp.max(s, axis=-1, keepdims=True)
        p = jnp.exp(s - m)
        l = jnp.sum(p, axis=-1, keepdims=True)
        o = jnp.dot(p.astype(jnp.bfloat16), v, preferred_element_type=jnp.float32)
        o_ref[h] = (o / l).astype(o_ref.dtype)


@jax.jit
def pallas_standalone__mha_softmax__near_ridge_kernel(
    q: jax.Array,
    k: jax.Array,
    v: jax.Array,
):
    B, H, Sq, D = q.shape
    Sk = k.shape[2]
    BH = B * H
    hb = 4
    scale = float(D) ** -0.5
    q3 = q.reshape(BH, Sq, D)
    k3 = k.reshape(BH, Sk, D)
    v3 = v.reshape(BH, Sk, D)
    out = pl.pallas_call(
        functools.partial(_mha_kernel, hb=hb, scale=scale),
        grid=(BH // hb,),
        in_specs=[
            pl.BlockSpec((hb, Sq, D), lambda i: (i, 0, 0)),
            pl.BlockSpec((hb, Sk, D), lambda i: (i, 0, 0)),
            pl.BlockSpec((hb, Sk, D), lambda i: (i, 0, 0)),
        ],
        out_specs=pl.BlockSpec((hb, Sq, D), lambda i: (i, 0, 0)),
        out_shape=jax.ShapeDtypeStruct((BH, Sq, D), q.dtype),
        compiler_params=pltpu.CompilerParams(
            dimension_semantics=("parallel",),
        ),
    )(q3, k3, v3)
    return out.reshape(B, H, Sq, D)
```

```python
import functools

import jax
import jax.numpy as jnp
import jax.experimental.pallas as pl
import jax.experimental.pallas.tpu as pltpu


def _attend_one_head(q, k, v, scale):
    s = jax.lax.dot_general(
        q, k, (((1,), (1,)), ((), ())), preferred_element_type=jnp.float32
    )
    s = s.astype(q.dtype).astype(jnp.float32) * scale
    m = jnp.max(s, axis=-1, keepdims=True)
    p = jnp.exp(s - m)
    l = jnp.sum(p, axis=-1, keepdims=True)
    o = jnp.dot(p.astype(v.dtype), v, preferred_element_type=jnp.float32)
    return o / l


def _mha_kernel(
    q_hbm, k_hbm, v_hbm, o_hbm,
    qbuf, kbuf, vbuf, obuf, in_sems, out_sems,
    *, hb, nbuf, nchunks, scale,
):
    n_heads = nchunks * hb

    def in_copies(c, slot):
        return [
            pltpu.make_async_copy(
                src.at[pl.ds(c * hb, hb)], buf.at[slot], in_sems.at[slot * 3 + j]
            )
            for j, (src, buf) in enumerate(
                ((q_hbm, qbuf), (k_hbm, kbuf), (v_hbm, vbuf))
            )
        ]

    def out_copy(first_head, num_heads, sem_idx):
        return pltpu.make_async_copy(
            obuf.at[pl.ds(first_head, num_heads)],
            o_hbm.at[pl.ds(first_head, num_heads)],
            out_sems.at[sem_idx],
        )

    def compute_chunk(c, slot):
        for h in range(hb):
            o = _attend_one_head(
                qbuf[slot, h], kbuf[slot, h], vbuf[slot, h], scale
            )
            obuf[c * hb + h] = o.astype(obuf.dtype)

    for s in range(nbuf):
        for cp in in_copies(s, s):
            cp.start()

    def body(c, carry):
        slot = jax.lax.rem(c, nbuf)
        for cp in in_copies(c, slot):
            cp.wait()
        compute_chunk(c, slot)

        @pl.when(c + nbuf < nchunks)
        def _():
            for cp in in_copies(c + nbuf, slot):
                cp.start()

        return carry

    jax.lax.fori_loop(0, nchunks - 1, body, 0)

    last = nchunks - 1
    last_slot = last % nbuf
    for cp in in_copies(last, last_slot):
        cp.wait()

    if last > 0:
        out_copy(0, last * hb, 0).start()
    compute_chunk(last, last_slot)
    out_copy(last * hb, n_heads - last * hb, 1).start()
    if last > 0:
        out_copy(0, last * hb, 0).wait()
    out_copy(last * hb, n_heads - last * hb, 1).wait()


@jax.jit
def pallas_standalone__mha_softmax__near_ridge_kernel(
    q: jax.Array,
    k: jax.Array,
    v: jax.Array,
):
    B, H, Sq, D = q.shape
    Sk = k.shape[2]
    Dv = v.shape[3]
    BH = B * H
    scale = float(D) ** -0.5

    hb = next(c for c in (8, 4, 2, 1) if BH % c == 0)
    nchunks = BH // hb
    nbuf = min(3, nchunks)

    any_spec = pl.BlockSpec(memory_space=pl.ANY)
    out = pl.pallas_call(
        functools.partial(
            _mha_kernel, hb=hb, nbuf=nbuf, nchunks=nchunks, scale=scale
        ),
        in_specs=[any_spec, any_spec, any_spec],
        out_specs=any_spec,
        out_shape=jax.ShapeDtypeStruct((BH, Sq, Dv), q.dtype),
        scratch_shapes=[
            pltpu.VMEM((nbuf, hb, Sq, D), q.dtype),
            pltpu.VMEM((nbuf, hb, Sk, D), k.dtype),
            pltpu.VMEM((nbuf, hb, Sk, Dv), v.dtype),
            pltpu.VMEM((BH, Sq, Dv), q.dtype),
            pltpu.SemaphoreType.DMA((nbuf * 3,)),
            pltpu.SemaphoreType.DMA((2,)),
        ],
        compiler_params=pltpu.CompilerParams(
            vmem_limit_bytes=64 * 1024 * 1024,
        ),
    )(
        q.reshape(BH, Sq, D),
        k.reshape(BH, Sk, D),
        v.reshape(BH, Sk, Dv),
    )
    return out.reshape(B, H, Sq, Dv)
```
